```python
import os as _os
_os.environ.setdefault('JAX_PLATFORMS', 'cpu')
import jax
import jax.numpy as jnp

def _softmax(x, axis=-1):
    return jax.nn.softmax(x, axis=axis)

def _gelu(x):
    return jax.nn.gelu(x, approximate=True)

def _silu(x):
    return jax.nn.silu(x)

def _sigmoid(x):
    return jax.nn.sigmoid(x)

def _layernorm(x, axis=-1, eps=1e-05):
    m = jnp.mean(x, axis=axis, keepdims=True)
    v = jnp.var(x, axis=axis, keepdims=True)
    return (x - m) / jnp.sqrt(v + eps)

def _scatter_add(tgt, idx, src, axis=0):
    return tgt.at[idx].add(src)

def _segment_sum(src, seg, n):
    return jax.ops.segment_sum(src, seg, n)

class _Rng:

    def __init__(self, key):
        self._k = key

    def _next(self):
        self._k, sub = jax.random.split(self._k)
        return sub

    def normal(self, shape):
        return jax.random.normal(self._next(), shape, dtype=jnp.bfloat16)

    def randint(self, lo, hi, shape):
        return jax.random.randint(self._next(), shape, lo, hi, dtype=jnp.int32)

    def uniform(self, shape, lo=0.0, hi=1.0):
        return jax.random.uniform(self._next(), shape, jnp.bfloat16, lo, hi)

    def permutation(self, n):
        return jax.random.permutation(self._next(), n)
kernel_name = 'gated_mix__memory_aug_recurrent_mem_tr__glu_gated_geglu__prompt'

def setup_inputs():
    _rng = _Rng(jax.random.key(int.from_bytes(__import__("os").urandom(4), "little")))
    _w = lambda a: (lambda t: t.astype(jnp.bfloat16) if jnp.issubdtype(t.dtype, jnp.floating) else t)(jnp.asarray(a))

    def _A_setup():
        B, S, Dm = (1, 2048, 640)
        H, Dh = (32, 128)
        M, seg = (8, 32)
        seg = min(seg, S)
        S = S // seg * seg
        return {'x': _w((lambda *s: _rng.normal(s) * 0.05)(B, S, Dm)), 'mem0': _w((lambda *s: _rng.normal(s) * 0.4)(B, M, Dm)), 'Wq': _w((lambda *s: _rng.normal(s) * 3.2)(Dm, H, Dh) * Dm ** (-0.5)), 'Wk': _w((lambda *s: _rng.normal(s) * 3.2)(Dm, H, Dh) * Dm ** (-0.5)), 'Wv': _w((lambda *s: _rng.normal(s) * 0.4)(Dm, H, Dh) * Dm ** (-0.5)), 'Wo': _w((lambda *s: _rng.normal(s) * 0.4)(H, Dh, Dm) * (H * Dh) ** (-0.5)), 'seg_len': seg}
    _A_in = _A_setup()

    def _B_setup():
        B, S, Dm, Df = (1, 2048, 640, 1728)
        return {'x': _w((lambda *s: _rng.normal(s) * 0.05)(B, S, Dm)), 'w_gate': _w((lambda *s: _rng.normal(s) * 1.6)(Dm, Df) * Dm ** (-0.5)), 'w_up': _w((lambda *s: _rng.normal(s) * 1.6)(Dm, Df) * Dm ** (-0.5)), 'w_down': _w((lambda *s: _rng.normal(s) * 1.6)(Df, Dm) * Df ** (-0.5))}
    _B_in = _B_setup()
    return {'A_x': _A_in['x'], 'A_mem0': _A_in['mem0'], 'A_Wq': _A_in['Wq'], 'A_Wk': _A_in['Wk'], 'A_Wv': _A_in['Wv'], 'A_Wo': _A_in['Wo'], 'A_seg_len': _A_in['seg_len'], 'B_x': _B_in['x'], 'B_w_gate': _B_in['w_gate'], 'B_w_up': _B_in['w_up'], 'B_w_down': _B_in['w_down'], 'gate_w': _w((lambda *s: _rng.normal(s) * 0.05)(640) * 16.0)}

def reference(A_x, A_mem0, A_Wq, A_Wk, A_Wv, A_Wo, A_seg_len, B_x, B_w_gate, B_w_up, B_w_down, gate_w):

    def _A_ref(x, mem0, Wq, Wk, Wv, Wo, seg_len):
        B, S, Dm = x.shape
        H, Dh = (Wq.shape[1], Wq.shape[2])
        M = mem0.shape[1]
        scale = Dh ** (-0.5)
        n_seg = S // seg_len
        L = M + seg_len
        idx = jnp.arange(L)
        mask = (idx[:, None] < M) | (idx[:, None] >= idx[None, :])
        mem = mem0
        outs = []
        for s in range(n_seg):
            xs = x[:, s * seg_len:(s + 1) * seg_len, :].copy()
            h = jnp.concatenate([mem, xs], axis=1)
            q = jnp.einsum('btd,dhe->bhte', h, Wq)
            k = jnp.einsum('btd,dhe->bhte', h, Wk)
            v = jnp.einsum('btd,dhe->bhte', h, Wv)
            scores = jnp.einsum('bhqe,bhke->bhqk', q, k) * scale
            scores = jnp.where(mask[None, None], scores, -1000000000.0)
            p = _softmax(scores, axis=-1)
            o = jnp.einsum('bhqk,bhke->bhqe', p, v)
            o = jnp.einsum('bhte,hed->btd', o, Wo)
            mem = o[:, :M, :].copy()
            outs.append(o[:, M:, :])
        return jnp.concatenate(outs, axis=1)

    def _B_ref(x, w_gate, w_up, w_down):
        g = jnp.einsum('bsd,df->bsf', x, w_gate)
        u = jnp.einsum('bsd,df->bsf', x, w_up)
        h = _gelu(g) * u
        return jnp.einsum('bsf,fd->bsd', h, w_down)
    x = A_x
    g = _sigmoid((x * gate_w).sum(-1, keepdims=True))
    a = _A_ref(x, A_mem0, A_Wq, A_Wk, A_Wv, A_Wo, A_seg_len)
    b = _B_ref(x, B_w_gate, B_w_up, B_w_down)
    return g * a + (1 - g) * b
```

```python
import functools
import jax, jax.numpy as jnp, numpy as np
from jax.experimental import pallas as pl
from jax.experimental.pallas import tpu as pltpu

S, D, H, E, M, SEG, F = 2048, 640, 32, 128, 8, 32, 1728
L = M + SEG
NSEG = S // SEG
f32, bf16 = jnp.float32, jnp.bfloat16
u32 = jnp.uint32
PB = 256
PB0 = 512
FP = 1792
P = 2048
NCH = 7
G, D1, D2, D3 = 4, 1, 2, 3

def b16(w):
    return pltpu.bitcast(w, bf16)

def mm(a, b):
    return jax.lax.dot_general(a, b, (((1,), (0,)), ((), ())), preferred_element_type=f32)

def nt(a, b):
    return jax.lax.dot_general(a, b, (((1,), (1,)), ((), ())), preferred_element_type=f32)

def kern(x_hbm, mem_ref, gw_ref, wq_hbm, wk_hbm, wv_hbm, wo_hbm, wg_hbm, wu_hbm, wd_hbm, o_hbm,
         wqkv, stage, sems, wo_ref, wg_ref, wu_ref, wd_ref, bs, wsem, x_ref, o_ref, osem):
    srcs = (wq_hbm, wk_hbm, wv_hbm)
    wc = [pltpu.make_async_copy(a, b, wsem.at[i]) for i, (a, b) in enumerate(
        ((wg_hbm.bitcast(u32), wg_ref), (wu_hbm.bitcast(u32), wu_ref), (wd_hbm.bitcast(u32), wd_ref), (wo_hbm.bitcast(u32), wo_ref), (x_hbm.at[:PB0], x_ref.at[:PB0]), (x_hbm.at[PB0:], x_ref.at[PB0:])))]
    class cp:
        def __init__(self, t, c):
            self.cs = [pltpu.make_async_copy(srcs[t].bitcast(u32).at[:, c * 4 + i, :], stage.at[t * 16 + c * 4 + i],
                                             sems.at[t * 16 + c * 4 + i]) for i in range(4)]
        def start(self):
            for c in self.cs: c.start()
        def wait(self):
            for c in self.cs: c.wait()
    wc[4].start(); wc[0].start()
    gw = gw_ref[...].astype(f32)

    def glu(i, fill=lambda t: None, PB=PB):
        r = pl.multiple_of(i * PB, PB)
        fill(0)
        xb = x_ref[pl.ds(r, PB), :]
        gg = jax.nn.gelu(nt(xb, b16(wg_ref[...])), approximate=True)
        fill(1)
        hh = (gg * nt(xb, b16(wu_ref[...]))).astype(bf16)
        fill(2)
        bs[pl.ds(r, PB), :] = mm(hh, b16(wd_ref[...]))
    npb = P // PB
    def pro1(i, _):
        glu(i)
    def fill0(t):
        if t == 0:
            wc[4].wait(); wc[0].wait()
            wc[1].start(); wc[2].start(); wc[5].start()
        elif t == 1:
            wc[1].wait()
        else:
            wc[2].wait(); wc[5].wait()
            for c in range(2):
                for t2 in range(3):
                    cp(t2, c).start()
    glu(0, fill0, PB0)
    jax.lax.fori_loop(PB0 // PB, npb - 4, pro1, None)
    def pro2(c, _):
        for t in range(3):
            cp(t, c).wait()
        @pl.when(c == 0)
        def _():
            for c2 in (2, 3):
                for t in range(3):
                    cp(t, c2).start()
            wc[3].start()
        def fill(t):
            for i in range(4):
                wa = stage[t * 16 + c * 4 + i, pl.ds(0, D // 2, stride=2), :]
                wb = stage[t * 16 + c * 4 + i, pl.ds(1, D // 2, stride=2), :]
                base = c * (24 * E) + (6 * i + t) * E
                wqkv[:, pl.ds(pl.multiple_of(base, E), E)] = (wa & u32(0xFFFF)) | (wb << 16)
                wqkv[:, pl.ds(pl.multiple_of(base + 3 * E, E), E)] = (wa >> 16) | (wb & u32(0xFFFF0000))
        glu(c + npb - 4, fill)
    jax.lax.fori_loop(0, 4, pro2, None)

    row = jax.lax.broadcasted_iota(jnp.int32, (L, L), 0)
    col = jax.lax.broadcasted_iota(jnp.int32, (L, L), 1)
    mask = (row < M) | (row >= col)
    scale = E ** -0.5

    def step(s, mem):
        r0 = pl.multiple_of(s * SEG, SEG)
        xs = x_ref[pl.ds(r0, SEG), :].astype(f32)
        h = jnp.concatenate([mem, xs], axis=0)
        NG = H // G; W = 3 * E * G
        ys, ps, os_ = {}, {}, {}
        acc = None
        for t in range(NG + D3):
            if t < NG:
                ys[t] = mm(h, b16(wqkv[:, t * W:(t + 1) * W]))
            g = t - D1
            if 0 <= g < NG:
                for i in range(G):
                    y = ys[g]
                    sc = nt(y[:, 3 * i * E:(3 * i + 1) * E], y[:, (3 * i + 1) * E:(3 * i + 2) * E])
                    sc = jnp.where(mask, sc * scale, -1e9)
                    p = jnp.exp(sc - jnp.max(sc, axis=-1, keepdims=True))
                    ps[g, i] = (p, jnp.sum(p, axis=-1, keepdims=True))
            g = t - D2
            if 0 <= g < NG:
                os_[g] = jnp.concatenate([mm(ps[g, i][0], ys[g][:, (3 * i + 2) * E:(3 * i + 3) * E]) / ps[g, i][1] for i in range(G)], axis=1)
            g = t - D3
            if 0 <= g < NG:
                z = mm(os_[g], b16(wo_ref[g * G * E // 2:(g + 1) * G * E // 2, :]))
                acc = z if acc is None else acc + z
        b = bs[pl.ds(r0, SEG), :]
        gate = jax.nn.sigmoid(jnp.sum(xs * gw, axis=-1, keepdims=True))
        o_ref[pl.ds(r0, SEG), :] = (gate * acc[M:] + (1 - gate) * b).astype(o_ref.dtype)
        return acc[:M].astype(bf16).astype(f32)
    wc[3].wait()
    OC = 8
    def ocp(i):
        rows = pl.ds(pl.multiple_of(i * (S // OC), S // OC), S // OC)
        return pltpu.make_async_copy(o_ref.at[rows], o_hbm.at[rows], osem.at[i])
    def step2(s, mem):
        mem = step(s, mem)
        @pl.when(s % (NSEG // OC) == NSEG // OC - 1)
        def _():
            ocp(s // (NSEG // OC)).start()
        return mem
    jax.lax.fori_loop(0, NSEG, step2, mem_ref[...].astype(f32))
    for i in range(OC):
        ocp(i).wait()

@jax.jit
def pallas_gated_mix__memory_aug_recurrent_mem_tr__glu_gated_geglu__prompt_kernel(
        A_x, A_mem0, A_Wq, A_Wk, A_Wv, A_Wo, A_seg_len, B_x, B_w_gate, B_w_up, B_w_down, gate_w):
    vm = pl.BlockSpec(memory_space=pltpu.VMEM)
    anyspec = pl.BlockSpec(memory_space=pl.ANY)
    out = pl.pallas_call(
        kern,
        out_shape=jax.ShapeDtypeStruct((S, D), bf16),
        in_specs=[anyspec, vm, vm] + [anyspec] * 7,
        out_specs=anyspec,
        scratch_shapes=[pltpu.VMEM((D // 2, 3 * H * E), u32), pltpu.VMEM((48, D, E), u32), pltpu.SemaphoreType.DMA((48,)),
                        pltpu.VMEM((H * E // 2, D), u32), pltpu.VMEM((F // 2, D), u32), pltpu.VMEM((F // 2, D), u32), pltpu.VMEM((F // 2, D), u32),
                        pltpu.VMEM((S, D), f32), pltpu.SemaphoreType.DMA((6,)), pltpu.VMEM((S, D), bf16), pltpu.VMEM((S, D), bf16),
                        pltpu.SemaphoreType.DMA((8,))],
        compiler_params=pltpu.CompilerParams(vmem_limit_bytes=100 * 2**20),
    )(A_x.reshape(S, D), A_mem0.reshape(M, D), gate_w.reshape(1, D), A_Wq, A_Wk, A_Wv,
      A_Wo.reshape(H * E, D), B_w_gate.T, B_w_up.T, B_w_down)
    return out.reshape(1, S, D)
```
